```python
import os as _os
_os.environ.setdefault("JAX_PLATFORMS", "cpu")
import jax
import jax.numpy as jnp

def _softmax(x, axis=-1):
    return jax.nn.softmax(x, axis=axis)
def _gelu(x):
    return jax.nn.gelu(x, approximate=True)
def _silu(x):
    return jax.nn.silu(x)
def _sigmoid(x):
    return jax.nn.sigmoid(x)
def _layernorm(x, axis=-1, eps=1e-5):
    m = jnp.mean(x, axis=axis, keepdims=True)
    v = jnp.var(x, axis=axis, keepdims=True)
    return (x - m) / jnp.sqrt(v + eps)
def _scatter_add(tgt, idx, src, axis=0):
    return tgt.at[idx].add(src)
def _segment_sum(src, seg, n):
    return jax.ops.segment_sum(src, seg, n)
class _Rng:
    def __init__(self, key):
        self._k = key
    def _next(self):
        self._k, sub = jax.random.split(self._k)
        return sub
    def normal(self, shape):
        return jax.random.normal(self._next(), shape, dtype=jnp.bfloat16)
    def randint(self, lo, hi, shape):
        return jax.random.randint(self._next(), shape, lo, hi, dtype=jnp.int32)
    def uniform(self, shape, lo=0.0, hi=1.0):
        return jax.random.uniform(self._next(), shape, jnp.bfloat16, lo, hi)
    def permutation(self, n):
        return jax.random.permutation(self._next(), n)


kernel_name = 'gated_mix__sliding_block__sliding_local_dilated__prompt'

def setup_inputs():
    _rng = _Rng(jax.random.key(int.from_bytes(__import__("os").urandom(4), "little")))
    _w = (lambda a: (lambda t: t.astype(jnp.bfloat16) if jnp.issubdtype(t.dtype, jnp.floating) else t)(jnp.asarray(a)))
    def _A_setup():
        B, S, D = 1, 2048, 640
        return {
            "x": _w((lambda *s: _rng.normal(s) * 0.05)(B, S, D)),
            "wqkv": _w((lambda *s: _rng.normal(s) * 0.8)(D, 3 * D)),
            "wo": _w((lambda *s: _rng.normal(s) * 0.05)(D, D)),
        }
    _A_in = _A_setup()

    def _B_setup():
        B, S, D = 1, 2048, 640
        return {
            "x": _w((lambda *s: _rng.normal(s) * 0.05)(B, S, D)),
            "wqkv": _w((lambda *s: _rng.normal(s) * 0.8)(D, 3 * D)),
            "wo": _w((lambda *s: _rng.normal(s) * 0.05)(D, D)),
        }
    _B_in = _B_setup()

    return {
        "A_x": _A_in["x"],
        "A_wqkv": _A_in["wqkv"],
        "A_wo": _A_in["wo"],
        "B_x": _B_in["x"],
        "B_wqkv": _B_in["wqkv"],
        "B_wo": _B_in["wo"],
        "gate_w": _w((lambda *s: _rng.normal(s) * 0.05)(640) * 16.0),
    }

def reference(A_x, A_wqkv, A_wo, B_x, B_wqkv, B_wo, gate_w):
    def _A_ref(x, wqkv, wo):
        B, S, D = x.shape
        H = 32; Dh = D // H; W = 256
        qkv = (lambda x, *d: x.transpose(*d))((x @ wqkv).reshape(B, S, 3, H, Dh), 2, 0, 3, 1, 4)
        q, k, v = qkv[0], qkv[1], qkv[2]
        scores = jnp.einsum("bhqd,bhkd->bhqk", q, k) * (Dh ** -0.5)
        idx = jnp.arange(S)
        mask = (idx[:, None] - idx[None, :] >= 0) & (idx[:, None] - idx[None, :] < W)
        scores = jnp.where(mask[None, None], scores, -1e9)
        p = _softmax(scores, axis=-1)
        o = jnp.einsum("bhqk,bhkd->bhqd", p, v)
        return (lambda x, *d: x.transpose(*d))(o, 0, 2, 1, 3).reshape(B, S, D) @ wo

    def _B_ref(x, wqkv, wo):
        B, S, D = x.shape
        H = 32; Dh = D // H
        W, dil = 8, 2
        qkv = (lambda x, *d: x.transpose(*d))((x @ wqkv).reshape(B, S, 3, H, Dh), 2, 0, 3, 1, 4)
        q, k, v = qkv[0], qkv[1], qkv[2]
        scale = Dh ** -0.5
        pos = jnp.arange(S)
        off = jnp.arange(W) * dil
        idx = pos[:, None] - off[None, :]
        mask = idx >= 0
        idx_c = jnp.where(mask, idx, 0).reshape(-1)
        kg = k[:, :, idx_c, :].reshape(B, H, S, W, Dh)
        vg = v[:, :, idx_c, :].reshape(B, H, S, W, Dh)
        logits = jnp.einsum("bhsd,bhswd->bhsw", q, kg) * scale
        logits = jnp.where(mask[None, None, :, :], logits, -1e9)
        attn = _softmax(logits, axis=-1)
        o = jnp.einsum("bhsw,bhswd->bhsd", attn, vg)
        return (lambda x, *d: x.transpose(*d))(o, 0, 2, 1, 3).reshape(B, S, D) @ wo

    x = A_x
    g = _sigmoid((x * gate_w).sum(-1, keepdims=True))
    a = _A_ref(x, A_wqkv, A_wo)
    b = _B_ref(x, B_wqkv, B_wo)
    return g * a + (1 - g) * b
```

```python
import functools
import math
import jax
import jax.numpy as jnp
from jax import lax
import jax.experimental.pallas as pl
import jax.experimental.pallas.tpu as pltpu

S, D, H, DH = 2048, 640, 32, 20
BQ = 256
RB = 16
NT = (((1,), (1,)), ((), ()))
LOG2E = 1.4426950408889634
QSCALE = (DH ** -0.5) * LOG2E
NEG = -1e30
f32, bf16 = jnp.float32, jnp.bfloat16

def _head_ranges():
    strad = {6: 0, 12: 32, 19: 64, 25: 96}
    out = []
    for h in range(H):
        lo, hi = DH * h, DH * h + DH
        if h in strad:
            r = strad[h]
            a, b = (lo % 128 + r) % 128, (hi % 128 + r) % 128
            out.append((5, a, b))
        else:
            out.append((lo // 128, lo % 128, lo % 128 + DH))
    return out
HEADS = _head_ranges()

def _with_aux(t):
    c = [t[:, 128 * i:128 * i + 128] for i in range(5)]
    lane = lax.broadcasted_iota(jnp.int32, c[0].shape, 1)
    m6 = jnp.where(lane >= 120, c[0], c[1])
    m12 = pltpu.roll(jnp.where(lane >= 112, c[1], c[2]), 32, 1)
    m19 = pltpu.roll(jnp.where(lane >= 124, c[2], c[3]), 64, 1)
    m25 = pltpu.roll(jnp.where(lane >= 116, c[3], c[4]), 96, 1)
    aux = jnp.where((lane >= 16) & (lane < 36), m12, m6)
    aux = jnp.where((lane >= 60) & (lane < 80), m19, aux)
    aux = jnp.where((lane >= 84) & (lane < 104), m25, aux)
    return c + [aux]

def kernel(ax_ref, wa_hbm, woa_hbm, wb_hbm, wob_hbm, gw_ref, out_ref,
           wa_ref, woa_ref, wb_ref, wob_ref, sems,
           ka_ref, vt_ref, wvt_ref, wbt_ref, wobp_ref, tmp_ref, qb_ref, kb_ref, vb_ref, oa_ref, ob_ref):
    i = pl.program_id(0)

    def copies():
        cs = [pltpu.make_async_copy(wa_hbm.at[:, t * D:(t + 1) * D], wa_ref.at[:, t * D:(t + 1) * D], sems.at[t]) for t in range(3)]
        cs += [pltpu.make_async_copy(wb_hbm.at[:, t * D:(t + 1) * D], wb_ref.at[:, t * D:(t + 1) * D], sems.at[3 + t]) for t in range(3)]
        cs += [pltpu.make_async_copy(wob_hbm, wob_ref, sems.at[6]), pltpu.make_async_copy(woa_hbm, woa_ref, sems.at[7])]
        return cs

    @pl.when(i == 0)
    def _init():
        for c in copies():
            c.start()
        kb_ref[:, 0:24, :] = jnp.zeros((4, 24, D), f32)
        vb_ref[:, 0:24, :] = jnp.zeros((4, 24, D), f32)

    @pl.when(i > 0)
    def _hist():
        kb_ref[:, 0:24, :] = kb_ref[:, BQ:BQ + 24, :]
        vb_ref[:, 0:24, :] = vb_ref[:, BQ:BQ + 24, :]

    def step(first):
        xa = ax_ref[0]
        row0 = pl.multiple_of(i * BQ, BQ)
        cs = copies()

        def permute_rows(dst_ref, r0, slot):
            for c in range(5):
                for d in range(DH):
                    dst_ref[r0 + 32 * d:r0 + 32 * d + 32, 128 * c:128 * c + 128] = (
                        tmp_ref.at[slot + c][pl.ds(d, 32, stride=DH), :].astype(bf16))

        def b_proj(t):
            if first:
                cs[3 + t].wait()
                for c in range(5):
                    tmp_ref[5 * t + c] = wb_ref[128 * c:128 * c + 128, t * D:(t + 1) * D].astype(f32).T
                permute_rows(wbt_ref, t * D, 5 * t)
            y = lax.dot_general(xa, wbt_ref[t * D:(t + 1) * D, :], NT, preferred_element_type=f32)
            if t == 0:
                qb_ref[...] = y * QSCALE
            else:
                dst = kb_ref if t == 1 else vb_ref
                for s_ in range(4):
                    dst[s_, 16 + 2 * s_:16 + 2 * s_ + BQ, :] = y

        def b_group(r):
            q = qb_ref[RB * r:RB * r + RB, :]
            lg = []
            for w in range(8):
                kk = kb_ref[w % 4, pl.ds(16 + RB * r - 8 * (w // 4), RB), :]
                pr = q * kk
                t = pr[:, 0:128] + pr[:, 128:256] + pr[:, 256:384] + pr[:, 384:512] + pr[:, 512:640]
                t = t + pltpu.roll(t, 64, 1)
                t = t + pltpu.roll(t, 32, 1)
                if first and RB * r < 16:
                    rr = lax.broadcasted_iota(jnp.int32, (RB, 128), 0) + RB * r
                    t = jnp.where(rr >= 2 * w, t, NEG)
                lg.append(t)
            mx = functools.reduce(jnp.maximum, lg)
            e = [jnp.exp2(t - mx) for t in lg]
            inv = 1.0 / functools.reduce(lambda a, b: a + b, e)
            acc = None
            for w in range(8):
                a = e[w] * inv
                a5 = jnp.concatenate([a] * 5, axis=1)
                vv = vb_ref[w % 4, pl.ds(16 + RB * r - 8 * (w // 4), RB), :]
                acc = a5 * vv if acc is None else acc + a5 * vv
            ob_ref[RB * r:RB * r + RB, :] = acc.astype(bf16)

        NG = BQ // RB

        def a_q():
            if first:
                cs[0].wait()
            qa = jnp.dot(xa, wa_ref[:, 0:D], preferred_element_type=f32) * QSCALE
            return [c.astype(bf16) for c in _with_aux(qa)]

        def a_k():
            if first:
                cs[1].wait()
            ka = jnp.dot(xa, wa_ref[:, D:2 * D], preferred_element_type=f32)
            kc = _with_aux(ka)
            for c in range(6):
                ka_ref[pl.ds(row0, BQ), 128 * c:128 * c + 128] = kc[c].astype(bf16)

        def a_v():
            if first:
                cs[2].wait()
                wvt_ref[...] = wa_ref[:, 2 * D:].astype(f32).T.astype(bf16)
            vt = lax.dot_general(wvt_ref[...], xa, NT, preferred_element_type=f32).astype(bf16)
            for j in range(BQ // 128):
                vt_ref[(BQ // 128) * i + j] = vt[:, 128 * j:128 * j + 128]

        if first:
            qc = a_q(); a_k(); a_v()
            bsched = {}
        else:
            for t in range(3):
                b_proj(t)
            bsched = {}
            k3 = [NG // 3, NG // 3, NG - 2 * (NG // 3)]
            for r in range(k3[0]): b_group(r)
            qc = a_q()
            for r in range(k3[0], k3[0] + k3[1]): b_group(r)
            a_k()
            for r in range(k3[0] + k3[1], NG): b_group(r)
            a_v()

        lane = lax.broadcasted_iota(jnp.int32, (128, 128), 1)
        krow = lax.broadcasted_iota(jnp.int32, (128, 128), 0)
        tri = krow <= lane
        trim = pltpu.bitcast(jnp.where(tri, 1.0, 0.0).astype(bf16), jnp.int32)
        trim = jnp.where((trim & 0xFFFF) != 0, 0xFFFF, 0) | jnp.where((trim >> 16) != 0, -65536, 0)
        sub8 = lax.broadcasted_iota(jnp.int32, (8, 128), 0)

        units = [(j, h) for j in range(BQ // 128) for h in range(H)]
        st = {}
        prev = [None]
        def qk(u):
            j, h = u
            qblk = (BQ // 128) * i + j
            nt = min(j + 1, 3) if first else 3
            kstart = pl.multiple_of((qblk - (nt - 1)) * 128, 128)
            c, lo, hi = HEADS[h]
            if lo < hi:
                msk = (lane >= lo) & (lane < hi)
            else:
                msk = (lane >= lo) | (lane < hi)
            qm = jnp.where(msk, qc[c][128 * j:128 * j + 128, :], jnp.zeros((128, 128), bf16))
            kk = ka_ref[pl.ds(kstart, nt * 128), 128 * c:128 * c + 128]
            st[u] = lax.dot_general(kk, qm, NT, preferred_element_type=f32)
        def smx(u):
            j, h = u
            nt = min(j + 1, 3) if first else 3
            s = st[u]
            s2 = s[(nt - 1) * 128:]
            p0 = p1 = None
            if nt == 3:
                sm = jnp.where(tri, s2, s[0:128])
            else:
                sm = jnp.where(tri, s2, NEG)
            if nt >= 2:
                s1 = s[(nt - 2) * 128:(nt - 1) * 128]
                mx = jnp.max(jnp.maximum(sm, s1), axis=0, keepdims=True)
            else:
                mx = jnp.max(sm, axis=0, keepdims=True)
            pm = jnp.exp2(sm - mx)
            pmi = pltpu.bitcast(pm.astype(bf16), jnp.int32)
            p2 = pltpu.bitcast(pmi & trim, bf16)
            if nt >= 2:
                p1 = jnp.exp2(s1 - mx)
                l = jnp.sum(pm + p1, axis=0, keepdims=True)
                p1 = p1.astype(bf16)
            else:
                l = jnp.sum(pm, axis=0, keepdims=True)
            if nt == 3:
                p0 = pltpu.bitcast(pmi & ~trim, bf16)
            st[u] = (p0, p1, p2, l)
        def pv(u):
            j, h = u
            qblk = (BQ // 128) * i + j
            p0, p1, p2, l = st[u]
            base = (DH * h // 16) * 16
            o = jnp.dot(vt_ref[qblk, base:base + 32, :], p2, preferred_element_type=f32)
            if p1 is not None:
                o = o + jnp.dot(vt_ref[qblk - 1, base:base + 32, :], p1, preferred_element_type=f32)
            if p0 is not None:
                o = o + jnp.dot(vt_ref[qblk - 2, base:base + 32, :], p0, preferred_element_type=f32)
            st[u] = (o, l)
        def fin(u):
            j, h = u
            o, l = st[u]
            base = (DH * h // 16) * 16
            o = o * (1.0 / l)
            off = DH * h - base
            if h % 2 == 0:
                g0 = off // 8
                oa_ref[j, DH * h:DH * h + 16, :] = o[8 * g0:8 * g0 + 16]
                prev[0] = o[8 * g0 + 16:8 * g0 + 24]
            else:
                g0 = (off - 4) // 8
                oa_ref[j, DH * h - 4:DH * h + 4, :] = jnp.where(sub8 < 4, prev[0], o[8 * g0:8 * g0 + 8])
                oa_ref[j, DH * h + 4:DH * h + 20, :] = o[8 * g0 + 8:8 * g0 + 24]
        n = len(units)
        for t in range(n + 8):
            for r in bsched.get(t, []): b_group(r)
            if t < n: qk(units[t])
            if 0 <= t - 4 < n: smx(units[t - 4])
            if 0 <= t - 6 < n: pv(units[t - 6])
            if 0 <= t - 8 < n: fin(units[t - 8])

        if first:
            for t in range(3):
                b_proj(t)
            cs[6].wait()
            for c in range(5):
                tmp_ref[15 + c] = wob_ref[:, 128 * c:128 * c + 128].astype(f32)
            permute_rows(wobp_ref, 0, 15)
            cs[7].wait()
            for r in range(NG): b_group(r)
        g = jax.nn.sigmoid(jnp.sum(xa.astype(f32) * gw_ref[...].astype(f32).reshape(1, D), axis=1, keepdims=True))
        oa = jnp.concatenate([oa_ref[j].T for j in range(BQ // 128)], axis=0).astype(bf16)
        a = jnp.dot(oa, woa_ref[...], preferred_element_type=f32)
        b = jnp.dot(ob_ref[...], wobp_ref[...], preferred_element_type=f32)
        out_ref[0] = (b + g * (a - b)).astype(out_ref.dtype)

    @pl.when(i == 0)
    def _():
        step(True)

    @pl.when(i > 0)
    def _():
        step(False)


@jax.jit
def pallas_gated_mix__sliding_block__sliding_local_dilated__prompt_kernel(A_x, A_wqkv, A_wo, B_x, B_wqkv, B_wo, gate_w):
    xspec = pl.BlockSpec((1, BQ, D), lambda i: (0, i, 0))
    hbm = pl.BlockSpec(memory_space=pl.ANY)
    return pl.pallas_call(
        kernel,
        grid=(S // BQ,),
        in_specs=[xspec, hbm, hbm, hbm, hbm, pl.BlockSpec((D,), lambda i: (0,))],
        out_specs=xspec,
        out_shape=jax.ShapeDtypeStruct((1, S, D), A_x.dtype),
        scratch_shapes=[
            pltpu.VMEM((D, 3 * D), bf16),
            pltpu.VMEM((D, D), bf16),
            pltpu.VMEM((D, 3 * D), bf16),
            pltpu.VMEM((D, D), bf16),
            pltpu.SemaphoreType.DMA((8,)),
            pltpu.VMEM((S, 768), bf16),
            pltpu.VMEM((S // 128, D, 128), bf16),
            pltpu.VMEM((D, D), bf16),
            pltpu.VMEM((3 * D, D), bf16),
            pltpu.VMEM((D, D), bf16),
            pltpu.VMEM((20, D, 128), f32),
            pltpu.VMEM((BQ, D), f32),
            pltpu.VMEM((4, BQ + 24, D), f32),
            pltpu.VMEM((4, BQ + 24, D), f32),
            pltpu.VMEM((BQ // 128, D, 128), f32),
            pltpu.VMEM((BQ, D), bf16),
        ],
        compiler_params=pltpu.CompilerParams(dimension_semantics=("arbitrary",), vmem_limit_bytes=100 * 1024 * 1024),
    )(A_x, A_wqkv, A_wo, B_wqkv, B_wo, gate_w)
```
